```python
import os as _os
_os.environ.setdefault("JAX_PLATFORMS", "cpu")
import jax
import jax.numpy as jnp

def _softmax(x, axis=-1):
    return jax.nn.softmax(x, axis=axis)
def _gelu(x):
    return jax.nn.gelu(x, approximate=True)
def _silu(x):
    return jax.nn.silu(x)
def _sigmoid(x):
    return jax.nn.sigmoid(x)
def _layernorm(x, axis=-1, eps=1e-5):
    m = jnp.mean(x, axis=axis, keepdims=True)
    v = jnp.var(x, axis=axis, keepdims=True)
    return (x - m) / jnp.sqrt(v + eps)
def _scatter_add(tgt, idx, src, axis=0):
    return tgt.at[idx].add(src)
def _segment_sum(src, seg, n):
    return jax.ops.segment_sum(src, seg, n)
class _Rng:
    def __init__(self, key):
        self._k = key
    def _next(self):
        self._k, sub = jax.random.split(self._k)
        return sub
    def normal(self, shape):
        return jax.random.normal(self._next(), shape, dtype=jnp.bfloat16)
    def randint(self, lo, hi, shape):
        return jax.random.randint(self._next(), shape, lo, hi, dtype=jnp.int32)
    def uniform(self, shape, lo=0.0, hi=1.0):
        return jax.random.uniform(self._next(), shape, jnp.bfloat16, lo, hi)
    def permutation(self, n):
        return jax.random.permutation(self._next(), n)


kernel_name = 'sequential_preLN__mha_block__swiglu_ffn__prompt'

def setup_inputs():
    _rng = _Rng(jax.random.key(int.from_bytes(__import__("os").urandom(4), "little")))
    _w = (lambda a: (lambda t: t.astype(jnp.bfloat16) if jnp.issubdtype(t.dtype, jnp.floating) else t)(jnp.asarray(a)))
    def _A_setup():
        B, S, D, H = 1, 2048, 640, 32
        return {
            "x": _w((lambda *s: _rng.normal(s) * 0.05)(B, S, D)),
            "wqkv": _w((lambda *s: _rng.normal(s) * 0.05)(D, 3 * D)),
            "wo": _w((lambda *s: _rng.normal(s) * 0.05)(D, D)),
        }
    _A_in = _A_setup()

    def _B_setup():
        B, S, D, F = 1, 2048, 640, 1728
        return {
            "x": _w((lambda *s: _rng.normal(s) * 0.05)(B, S, D)),
            "w_gate": _w((lambda *s: _rng.normal(s) * 0.05)(D, F)),
            "w_up": _w((lambda *s: _rng.normal(s) * 0.05)(D, F)),
            "w_down": _w((lambda *s: _rng.normal(s) * 0.05)(F, D)),
        }
    _B_in = _B_setup()

    return {
        "A_x": _A_in["x"],
        "A_wqkv": _A_in["wqkv"],
        "A_wo": _A_in["wo"],
        "B_x": _B_in["x"],
        "B_w_gate": _B_in["w_gate"],
        "B_w_up": _B_in["w_up"],
        "B_w_down": _B_in["w_down"],
    }

def reference(A_x, A_wqkv, A_wo, B_x, B_w_gate, B_w_up, B_w_down):
    def _A_ref(x, wqkv, wo):
        B, S, D = x.shape
        H = 32
        Dh = D // H
        qkv = (lambda x, *d: x.transpose(*d))((x @ wqkv).reshape(B, S, 3, H, Dh), 2, 0, 3, 1, 4)
        q, k, v = qkv[0], qkv[1], qkv[2]
        scores = jnp.einsum("bhqd,bhkd->bhqk", q, k) * (Dh ** -0.5)
        p = _softmax(scores, axis=-1)
        o = jnp.einsum("bhqk,bhkd->bhqd", p, v)
        return (lambda x, *d: x.transpose(*d))(o, 0, 2, 1, 3).reshape(B, S, D) @ wo

    def _B_ref(x, w_gate, w_up, w_down):
        g = _silu(x @ w_gate)
        u = x @ w_up
        return (g * u) @ w_down

    x = A_x
    h = x + _A_ref(_layernorm(x, axis=-1), A_wqkv, A_wo)
    h2 = h + _B_ref(_layernorm(h, axis=-1), B_w_gate, B_w_up, B_w_down)
    return h2
```

```python
import math
import jax
import jax.numpy as jnp
from jax import lax
import jax.experimental.pallas as pl
import jax.experimental.pallas.tpu as pltpu

S = 2048
D = 640
H = 32
DH = 20
FF = 1728
TQ = 512
CK = 128
NB = 4
NQB = S // TQ
NBLK = NQB * (H // NB)
TM1 = 512
TM3 = 256
FM = (FF // 128) * 128
FT = FF - FM
EPS = 1e-5
QSCALE = (DH ** -0.5) * math.log2(math.e)

BF = jnp.bfloat16
F32 = jnp.float32
NT = (((1,), (1,)), ((), ()))


def _layernorm(x):
    m = jnp.mean(x, axis=-1, keepdims=True)
    xc = x - m
    v = jnp.mean(xc * xc, axis=-1, keepdims=True)
    return xc * lax.rsqrt(v + EPS)


def _kernel(x_hbm, wqkv_hbm, wo_hbm, wg_hbm, wu_hbm, wd_hbm, out_hbm,
            x_v, wqkv_v, wo_v, wgu_v, wd_v, wqvt, kh, qt, vt,
            s0, s1, s2, s3, mbuf, ot, out_v, in_sems, out_sems):
    sbufs = (s0, s1, s2, s3)

    srcs = (x_hbm, wqkv_hbm, wo_hbm, wd_hbm,
            wg_hbm.at[pl.ds(0, FM), :], wu_hbm.at[pl.ds(0, FM), :],
            wg_hbm.at[pl.ds(FM, FT), :], wu_hbm.at[pl.ds(FM, FT), :])
    dsts = (x_v, wqkv_v, wo_v, wd_v,
            wgu_v.at[pl.ds(0, FM), :], wgu_v.at[pl.ds(FM, FM), :],
            wgu_v.at[pl.ds(2 * FM, FT), :], wgu_v.at[pl.ds(2 * FM + FT, FT), :])
    copies = [pltpu.make_async_copy(s_, d_, in_sems.at[i])
              for i, (s_, d_) in enumerate(zip(srcs, dsts))]
    copies[0].start()
    copies[1].start()
    copies[0].wait()
    copies[1].wait()
    for cp in copies[2:]:
        cp.start()

    wqvt[0:D, :] = wqkv_v[:, 0:D].astype(F32).T.astype(BF)
    wqvt[D:2 * D, :] = wqkv_v[:, 2 * D:3 * D].astype(F32).T.astype(BF)

    def proj_step(i, carry):
        r0 = pl.multiple_of(i * TM1, TM1)
        rows = pl.ds(r0, TM1)
        xn = _layernorm(x_v[rows, :].astype(F32)).astype(BF)
        k = jnp.dot(xn, wqkv_v[:, D:2 * D], preferred_element_type=F32).astype(BF)
        k32 = pltpu.bitcast(k, jnp.uint32)
        prow = pl.ds(pl.multiple_of(i * (TM1 // 2), TM1 // 2), TM1 // 2)
        lane = lax.broadcasted_iota(jnp.int32, (TM1 // 2, 128), 1)
        for h in range(H):
            w0 = (DH * h // 16) * 16
            g, rho = w0 // 128, w0 % 128
            src = k32[:, g * 128:(g + 1) * 128]
            if rho + 32 > 128:
                src = jnp.where(lane >= 64, src, k32[:, (g + 1) * 128:(g + 2) * 128])
            if rho:
                src = pltpu.roll(src, 128 - rho, 1)
            kh[h, prow, :] = src
        qv = lax.dot_general(wqvt[...], xn, NT, preferred_element_type=F32)
        row32 = lax.broadcasted_iota(jnp.int32, (32, TM1), 0)
        row24 = lax.broadcasted_iota(jnp.int32, (24, TM1), 0)
        for h in range(H):
            w0 = (DH * h // 16) * 16
            off = DH * h - w0
            qw = qv[w0:w0 + 32, :] * QSCALE
            qw = jnp.where((row32 >= off) & (row32 < off + DH), qw, 0.0)
            qt[h, :, rows] = qw.astype(BF)
            v0 = (DH * h // 8) * 8
            voff = DH * h - v0
            ones_row = DH if voff == 0 else 0
            vw = qv[D + v0:D + v0 + 24, :].astype(BF).astype(F32)
            vt[h, :, rows] = jnp.where(row24 == ones_row, 1.0, vw)
        return carry

    lax.fori_loop(0, S // TM1, proj_step, 0)

    nc = S // CK

    def item(b_cur, b_next, u, do_pv, do_qk):
        sbuf = sbufs[u]
        if do_pv:
            h = (b_cur % (H // NB)) * NB + u
            m_cur = mbuf[u]
        if do_qk:
            hn = (b_next % (H // NB)) * NB + u
            qn = pl.multiple_of((b_next // (H // NB)) * TQ, TQ)
            qw = qt[hn, :, pl.ds(qn, TQ)]
        acc = None
        mx = None
        for c in range(nc):
            sl = slice(c * CK, (c + 1) * CK)
            if do_qk:
                kc = pltpu.bitcast(kh[hn, c * (CK // 2):(c + 1) * (CK // 2), :], BF)
                s = jnp.dot(kc[:, 0:32], qw, preferred_element_type=F32)
            if do_pv:
                p = jnp.exp2(sbuf[sl, :] - m_cur).astype(BF)
                o = jnp.dot(vt[h, :, sl], p, preferred_element_type=F32)
                acc = o if acc is None else acc + o
            if do_qk:
                sbuf[sl, :] = s
                cm = jnp.max(s.reshape(CK // 8, 8, TQ), axis=0)
                mx = cm if mx is None else jnp.maximum(mx, cm)
        if do_qk:
            mbuf[u] = jnp.max(mx, axis=0, keepdims=True)
        if do_pv:
            ones_row = DH if u % 2 == 0 else 0
            return acc * (1.0 / acc[ones_row:ones_row + 1, :])
        return None

    def block(b_cur, b_next, do_pv, do_qk):
        res = [item(b_cur, b_next, u, do_pv, do_qk) for u in range(NB)]
        if do_pv:
            q0 = pl.multiple_of((b_cur // (H // NB)) * TQ, TQ)
            base = (b_cur % (H // NB)) * (NB * DH)
            sub = lax.broadcasted_iota(jnp.int32, (8, TQ), 0)
            for pr in range(NB // 2):
                ev, od = res[2 * pr], res[2 * pr + 1]
                mid = jnp.where(sub < 4, ev[16:24, :], od[0:8, :])
                blk = jnp.concatenate([ev[0:16, :], mid, od[8:24, :]], axis=0)
                r0 = pl.multiple_of(base + pr * 2 * DH, 8)
                ot[pl.ds(r0, 2 * DH), pl.ds(q0, TQ)] = blk

    block(None, 0, False, True)

    def attn_step(b, carry):
        block(b, b + 1, True, True)
        return carry

    lax.fori_loop(0, NBLK - 1, attn_step, 0)
    block(NBLK - 1, None, True, False)

    for cp in copies[2:]:
        cp.wait()

    n3 = S // TM3

    def out_copy(i, slot):
        r0 = pl.multiple_of(i * TM3, TM3)
        return pltpu.make_async_copy(out_v.at[slot], out_hbm.at[pl.ds(r0, TM3), :],
                                     out_sems.at[slot])

    def ffn_step(i, carry):
        slot = i % 2
        r0 = pl.multiple_of(i * TM3, TM3)
        rows = pl.ds(r0, TM3)
        o = ot[:, rows].T.astype(BF)
        hres = x_v[rows, :].astype(F32) + jnp.dot(o, wo_v[...], preferred_element_type=F32)
        hn = _layernorm(hres).astype(BF)
        gu = lax.dot_general(hn, wgu_v[...], NT, preferred_element_type=F32)
        g = gu[:, 0:FM]
        act = (g * jax.nn.sigmoid(g) * gu[:, FM:2 * FM]).astype(BF)
        gt = gu[:, 2 * FM:2 * FM + FT]
        actt = (gt * jax.nn.sigmoid(gt) * gu[:, 2 * FM + FT:2 * FF]).astype(BF)
        y = (hres + jnp.dot(act, wd_v[0:FM, :], preferred_element_type=F32)
             + jnp.dot(actt, wd_v[FM:FF, :], preferred_element_type=F32))

        @pl.when(i >= 2)
        def _():
            out_copy(i - 2, slot).wait()

        out_v[slot] = y.astype(BF)
        out_copy(i, slot).start()
        return carry

    lax.fori_loop(0, n3, ffn_step, 0)
    out_copy(n3 - 2, (n3 - 2) % 2).wait()
    out_copy(n3 - 1, (n3 - 1) % 2).wait()


@jax.jit
def pallas_sequential_preLN__mha_block__swiglu_ffn__prompt_kernel(
    A_x: jax.Array,
    A_wqkv: jax.Array,
    A_wo: jax.Array,
    B_x: jax.Array,
    B_w_gate: jax.Array,
    B_w_up: jax.Array,
    B_w_down: jax.Array,
):
    del B_x
    x2 = A_x.reshape(S, D)
    any_spec = pl.BlockSpec(memory_space=pltpu.HBM)
    out = pl.pallas_call(
        _kernel,
        out_shape=jax.ShapeDtypeStruct((S, D), BF),
        in_specs=[any_spec] * 6,
        out_specs=any_spec,
        scratch_shapes=[
            pltpu.VMEM((S, D), BF),
            pltpu.VMEM((D, 3 * D), BF),
            pltpu.VMEM((D, D), BF),
            pltpu.VMEM((2 * FF, D), BF),
            pltpu.VMEM((FF, D), BF),
            pltpu.VMEM((2 * D, D), BF),
            pltpu.VMEM((H, S // 2, 128), jnp.uint32),
            pltpu.VMEM((H, 32, S), BF),
            pltpu.VMEM((H, 24, S), F32),
            pltpu.VMEM((S, TQ), F32),
            pltpu.VMEM((S, TQ), F32),
            pltpu.VMEM((S, TQ), F32),
            pltpu.VMEM((S, TQ), F32),
            pltpu.VMEM((NB, 1, TQ), F32),
            pltpu.VMEM((D, S), F32),
            pltpu.VMEM((2, TM3, D), BF),
            pltpu.SemaphoreType.DMA((8,)),
            pltpu.SemaphoreType.DMA((2,)),
        ],
        compiler_params=pltpu.CompilerParams(vmem_limit_bytes=110 * 1024 * 1024),
    )(x2, A_wqkv, A_wo, B_w_gate.T, B_w_up.T, B_w_down)
    return out.reshape(1, S, D)
```

```python
import math
import jax
import jax.numpy as jnp
from jax import lax
import jax.experimental.pallas as pl
import jax.experimental.pallas.tpu as pltpu

S = 2048
D = 640
H = 32
DH = 20
FF = 1728
TQ = 512
CK = 128
NC = S // CK
NU = S // TQ
TM1 = 512
TM3 = 256
FM = (FF // 128) * 128
FT = FF - FM
EPS = 1e-5
QSCALE = (DH ** -0.5) * math.log2(math.e)

VG = (0, 8)
MG = tuple(g for g in range(15, -1, -1) if g not in VG)
KPERM = MG + VG
NKB = NC * len(VG) * DH
NQB = NU * DH * (TQ // 128)
NM = 3

BF = jnp.bfloat16
F32 = jnp.float32
U32 = jnp.uint32
NT = (((1,), (1,)), ((), ()))
HI16 = 0xFFFF0000
ONE_BF16_PAIR = 0x3F803F80
ACC_LIMIT = 2.0 ** 100
L_MAX = 2.0 ** 80
L_MIN = 2.0 ** -60


def _layernorm(x):
    m = jnp.mean(x, axis=-1, keepdims=True)
    xc = x - m
    v = jnp.mean(xc * xc, axis=-1, keepdims=True)
    return xc * lax.rsqrt(v + EPS)


def _layernorm_bf16(x, chunk=64):
    parts = [_layernorm(x[r:r + chunk, :]).astype(BF) for r in range(0, x.shape[0], chunk)]
    return jnp.concatenate(parts, axis=0)


def _row_slice(i, n):
    if isinstance(i, int):
        return slice(i * n, (i + 1) * n)
    return pl.ds(pl.multiple_of(i * n, n), n)


def _kbi(c, j, d):
    return (c * len(VG) + j) * DH + d


def _qbi(u, d, l):
    return NKB + (u * DH + d) * (TQ // 128) + l


def _lane_window(arr, start, lane):
    g, rho = start // 128, start % 128
    src = arr[:, g * 128:(g + 1) * 128]
    if rho + 32 > 128 and g + 1 < D // 128:
        src = jnp.where(lane >= 64, src, arr[:, (g + 1) * 128:(g + 2) * 128])
    if rho:
        src = pltpu.roll(src, 128 - rho, 1)
    return src


def _split_offset(m):
    terms = []
    rest = m
    for _ in range(NM):
        t = rest.astype(BF).astype(F32)
        terms.append(t)
        rest = rest - t
    tot = terms[0]
    for t in terms[1:]:
        tot = tot + t
    return terms, tot


def _fold_offset(qw, m, rstar, row32):
    terms, tot = _split_offset(m)
    for t_i, t in enumerate(terms):
        qw = jnp.where(row32 == rstar + t_i, -t, qw)
    return qw, -tot


def _kernel(x_hbm, wqkv_hbm, wo_hbm, wg_hbm, wu_hbm, wd_hbm, out_hbm,
            x_v, wqkv_v, wo_v, wgu_v, wd_v, xn_all, kperm, kcross, kh, kx, qa, negm, q32, vt,
            vb, fence, ctile, cacc, chk, otp, out_v, h_buf, hn_buf,
            x_sems, w_sems, out_sems):
    n1 = S // TM1

    def x_copy(i):
        rows = _row_slice(i, TM1) if not isinstance(i, int) else pl.ds(i * TM1, TM1)
        return pltpu.make_async_copy(x_hbm.at[rows, :], x_v.at[rows, :], x_sems.at[i])

    srcs = (wqkv_hbm.at[:, pl.ds(0, D)], wqkv_hbm.at[:, pl.ds(D, D)], wqkv_hbm.at[:, pl.ds(2 * D, D)],
            wo_hbm, wd_hbm,
            wg_hbm.at[pl.ds(0, FM), :], wu_hbm.at[pl.ds(0, FM), :],
            wg_hbm.at[pl.ds(FM, FT), :], wu_hbm.at[pl.ds(FM, FT), :])
    dsts = (wqkv_v.at[:, pl.ds(0, D)], wqkv_v.at[:, pl.ds(D, D)], wqkv_v.at[:, pl.ds(2 * D, D)],
            wo_v, wd_v,
            wgu_v.at[pl.ds(0, FM), :], wgu_v.at[pl.ds(FM, FM), :],
            wgu_v.at[pl.ds(2 * FM, FT), :], wgu_v.at[pl.ds(2 * FM + FT, FT), :])
    w_copies = [pltpu.make_async_copy(s_, d_, w_sems.at[i])
                for i, (s_, d_) in enumerate(zip(srcs, dsts))]
    WQ, WK, WV = 0, 1, 2
    x_copy(0).start()
    w_copies[WK].start()
    x_copy(0).wait()
    x_copy(1).start()

    def ln_rows(i):
        rows = _row_slice(i, TM1)
        xn_all[rows, :] = _layernorm_bf16(x_v[rows, :].astype(F32))

    ln_rows(0)
    w_copies[WK].wait()
    for i in range(2, n1):
        x_copy(i).start()
    w_copies[WQ].start()
    w_copies[WV].start()

    def k_step(i, carry):
        @pl.when(i + 1 < n1)
        def _():
            x_copy(i + 1).wait()

        k = jnp.dot(xn_all[_row_slice(i, TM1), :], wqkv_v[:, D:2 * D], preferred_element_type=F32)
        grp = lambda c, g: k[c * CK + g * 8:c * CK + g * 8 + 8, :]
        cpb = TM1 // CK
        kp = jnp.concatenate([grp(c, g) for c in range(cpb) for g in KPERM], axis=0).astype(BF)
        kperm[_row_slice(i, TM1 // 2), :] = pltpu.bitcast(kp, U32)
        lo = jnp.concatenate([grp(c, VG[0]) for c in range(cpb)], axis=0).astype(BF).astype(F32)
        hi = jnp.concatenate([grp(c, VG[1]) for c in range(cpb)], axis=0).astype(BF).astype(F32)
        kcross[_row_slice(i, cpb * 8), :] = ((pltpu.bitcast(lo, U32) >> 16)
                                             | (pltpu.bitcast(hi, U32) & jnp.uint32(HI16)))
        ln_rows(jnp.minimum(i + 1, n1 - 1))
        return carry

    lax.fori_loop(0, n1, k_step, 0)
    w_copies[WQ].wait()
    w_copies[WV].wait()
    for cp in w_copies[3:]:
        cp.start()

    def gen_kb(h, c):
        kk = kx[h, c * 8:(c + 1) * 8, :]
        for d in range(DH):
            w = jnp.broadcast_to(kk[:, d:d + 1], (8, 128))
            vb[_kbi(c, 0, d)] = w << 16
            vb[_kbi(c, 1, d)] = w & jnp.uint32(HI16)

    def gen_qb(h, u):
        for d in range(DH):
            qq = jnp.broadcast_to(q32[pl.ds(DH * h + d, 1), u * TQ:(u + 1) * TQ], (8, TQ))
            qq = pltpu.bitcast(qq, U32)
            for l in range(TQ // 128):
                vb[_qbi(u, d, l)] = qq[:, l * 128:(l + 1) * 128]

    def gen_first_head():
        for u in range(NU):
            gen_qb(0, u)
        for c in range(NC):
            gen_kb(0, c)

    def qv_step(i, carry):
        rows = _row_slice(i, TM1)
        xn = xn_all[rows, :]
        prow = _row_slice(i, TM1 // 2)
        xrow = _row_slice(i, TM1 // 16)
        kp = kperm[prow, :]
        kc = kcross[xrow, :]
        lane_p = lax.broadcasted_iota(jnp.int32, (TM1 // 2, 128), 1)
        lane_x = lax.broadcasted_iota(jnp.int32, (TM1 // 16, 128), 1)
        for h in range(H):
            w0 = (DH * h // 16) * 16
            rstar = (DH * h - w0 + DH) % 32
            win = _lane_window(kp, w0, lane_p)
            kh[h, prow, :] = jnp.where((lane_p >= rstar) & (lane_p < rstar + NM),
                                       jnp.uint32(ONE_BF16_PAIR), win)
            kx[h, xrow, :] = _lane_window(kc, DH * h, lane_x)
        q_t = jnp.dot(xn, wqkv_v[:, 0:D], preferred_element_type=F32).T
        q_t = (q_t * QSCALE).astype(BF).astype(F32)
        q32[:, rows] = q_t
        row32 = lax.broadcasted_iota(jnp.int32, (32, TM1), 0)
        row8 = lax.broadcasted_iota(jnp.int32, (8, TM1), 0)
        for h in range(H):
            w0 = (DH * h // 16) * 16
            off = DH * h - w0
            qw = jnp.where((row32 >= off) & (row32 < off + DH), q_t[w0:w0 + 32, :], 0.0)
            ksub = pltpu.bitcast(kh[h, 0:8, :], BF)[:, 0:32]
            msub = jnp.max(jnp.dot(ksub, qw.astype(BF), preferred_element_type=F32),
                           axis=0, keepdims=True)
            nm = jnp.broadcast_to(-(msub.astype(BF).astype(F32)), (8, TM1))
            rstar = (off + DH) % 32
            t0 = (rstar // 8) * 8
            tiles = [qw[r:r + 8, :] for r in range(0, 32, 8)]
            tiles[t0 // 8] = jnp.where(row8 == rstar - t0, nm, tiles[t0 // 8])
            qa[h, :, rows] = jnp.concatenate(tiles, axis=0).astype(BF)
            negm[h, :, rows] = nm
        if isinstance(i, int):
            gen_first_head()
        v_t = jnp.dot(xn, wqkv_v[:, 2 * D:3 * D], preferred_element_type=F32).T
        row24 = lax.broadcasted_iota(jnp.int32, (24, TM1), 0)
        for h in range(H):
            v0 = (DH * h // 8) * 8
            ones_row = DH if DH * h == v0 else 0
            vw = v_t[v0:v0 + 24, :].astype(BF).astype(F32)
            vt[h, :, rows] = jnp.where(row24 == ones_row, 1.0, vw)
        return carry

    lax.fori_loop(0, n1 - 1, qv_step, 0)
    qv_step(n1 - 1, 0)
    for cp in w_copies[3:]:
        cp.wait()

    def vpu_group(u, c, j, nm):
        accs = [nm[:, l * 128:(l + 1) * 128] for l in range(TQ // 128)]
        for d in range(DH):
            kb = pltpu.bitcast(vb[_kbi(c, j, d)], F32)
            for l in range(TQ // 128):
                accs[l] = accs[l] + kb * pltpu.bitcast(vb[_qbi(u, d, l)], F32)
        return jnp.concatenate(accs, axis=1)

    def pv_step(hh, u, c, tile, acc, never):
        p = jnp.exp2(tile).astype(BF)
        acc = acc + jnp.dot(vt[hh, :, c * CK:(c + 1) * CK], p, preferred_element_type=F32)
        if c == NC - 1:
            den = jnp.where(hh % 2 == 0, acc[DH:DH + 1, :], acc[0:1, :])
            otp[hh, :, u * TQ:(u + 1) * TQ] = acc * (1.0 / den)
            ok = (jnp.abs(acc) <= ACC_LIMIT) & (den <= L_MAX) & (den >= L_MIN)
            bad = jnp.where(ok, 0.0, 1.0)
            chk[...] = jnp.maximum(chk[...], jnp.maximum(jnp.maximum(bad[0:8], bad[8:16]), bad[16:24]))
            acc = jnp.where(never, acc, 0.0)
        return acc

    def head_step(h, carry):
        hp = (h + H - 1) % H
        hn = (h + 1) % H
        never = h < 0
        acc = cacc[...]
        pend = None
        for u in range(NU):
            cols = slice(u * TQ, (u + 1) * TQ)
            qw = qa[h, :, cols]
            nm = negm[h, :, cols]
            for c in range(NC):
                km = pltpu.bitcast(kh[h, c * 64:c * 64 + len(MG) * 4, :], BF)[:, 0:32]
                s = jnp.dot(km, qw, preferred_element_type=F32)
                g8 = {g: s[i * 8:(i + 1) * 8] for i, g in enumerate(MG)}
                for j, g in enumerate(VG):
                    g8[g] = vpu_group(u, c, j, nm)
                    fence[c % 8] = nm[:, 0:128]
                if u == NU - 1:
                    gen_kb(hn, c)
                if pend is None:
                    acc = pv_step(hp, NU - 1, NC - 1, ctile[...], acc, never)
                else:
                    acc = pv_step(h, pend[0], pend[1], pend[2], acc, never)
                pend = (u, c, jnp.concatenate([g8[g] for g in range(16)], axis=0))
            gen_qb(hn, u)
        ctile[...] = pend[2]
        cacc[...] = acc
        return carry

    def true_max_step(it, carry):
        h = it // NU
        cols = pl.ds(pl.multiple_of((it % NU) * TQ, TQ), TQ)
        rstar = ((4 * h) % 16 + DH) % 32
        row32 = lax.broadcasted_iota(jnp.int32, (32, TQ), 0)
        qw = qa[h, :, cols].astype(F32)
        qw = jnp.where((row32 >= rstar) & (row32 < rstar + NM), 0.0, qw)
        kall = pltpu.bitcast(kh[h], BF)[:, 0:32]
        m = jnp.max(jnp.dot(kall, qw.astype(BF), preferred_element_type=F32), axis=0, keepdims=True)
        qw, nm = _fold_offset(qw, m, rstar, row32)
        qa[h, :, cols] = qw.astype(BF)
        negm[h, :, cols] = jnp.broadcast_to(nm, (8, TQ))
        return carry

    def stage_a(i):
        rows = _row_slice(i, TM3)
        sub = lax.broadcasted_iota(jnp.int32, (8, TM3), 0)
        parts = []
        for pr in range(H // 2):
            ev = otp[2 * pr, :, rows]
            od = otp[2 * pr + 1, :, rows]
            parts += [ev[0:16, :], jnp.where(sub < 4, ev[16:24, :], od[0:8, :]), od[8:24, :]]
        o = jnp.concatenate(parts, axis=0).T.astype(BF)
        hres = x_v[rows, :].astype(F32) + jnp.dot(o, wo_v[...], preferred_element_type=F32)
        return hres, _layernorm_bf16(hres)

    def store_a(res):
        h_buf[...] = res[0]
        hn_buf[...] = res[1]

    def attention_pass(attempt, unsafe):
        @pl.when(unsafe > 0.0)
        def _():
            @pl.when(attempt > 0)
            def _():
                lax.fori_loop(0, H * NU, true_max_step, 0)

            ctile[...] = jnp.zeros(ctile.shape, F32)
            cacc[...] = jnp.ones(cacc.shape, F32)
            chk[...] = jnp.zeros(chk.shape, F32)
            lax.fori_loop(0, H, head_step, 0)
            pv_step(H - 1, NU - 1, NC - 1, ctile[...], cacc[...], attempt < 0)
            store_a(stage_a(0))

        return jnp.max(chk[...])

    chk[...] = jnp.zeros(chk.shape, F32)
    lax.fori_loop(0, 2, attention_pass, jnp.float32(1.0))

    n3 = S // TM3

    def out_copy(i, slot):
        r0 = pl.multiple_of(i * TM3, TM3)
        return pltpu.make_async_copy(out_v.at[slot], out_hbm.at[pl.ds(r0, TM3), :],
                                     out_sems.at[slot])


    def ffn_step(i, carry):
        slot = i % 2

        @pl.when(i >= 2)
        def _():
            out_copy(i - 2, slot).wait()

        gu = lax.dot_general(hn_buf[...], wgu_v[...], NT, preferred_element_type=F32)
        g = gu[:, 0:FM]
        act = (g * jax.nn.sigmoid(g) * gu[:, FM:2 * FM]).astype(BF)
        gt = gu[:, 2 * FM:2 * FM + FT]
        actt = (gt * jax.nn.sigmoid(gt) * gu[:, 2 * FM + FT:2 * FF]).astype(BF)
        nxt = stage_a(jnp.minimum(i + 1, n3 - 1))
        y = (h_buf[...] + jnp.dot(act, wd_v[0:FM, :], preferred_element_type=F32)
             + jnp.dot(actt, wd_v[FM:FF, :], preferred_element_type=F32))
        out_v[slot] = y.astype(BF)
        out_copy(i, slot).start()
        store_a(nxt)
        return carry

    lax.fori_loop(0, n3, ffn_step, 0)
    out_copy(n3 - 2, (n3 - 2) % 2).wait()
    out_copy(n3 - 1, (n3 - 1) % 2).wait()


@jax.jit
def pallas_sequential_preLN__mha_block__swiglu_ffn__prompt_kernel(
    A_x: jax.Array,
    A_wqkv: jax.Array,
    A_wo: jax.Array,
    B_x: jax.Array,
    B_w_gate: jax.Array,
    B_w_up: jax.Array,
    B_w_down: jax.Array,
):
    del B_x
    x2 = A_x.reshape(S, D)
    hbm_spec = pl.BlockSpec(memory_space=pltpu.HBM)
    out = pl.pallas_call(
        _kernel,
        out_shape=jax.ShapeDtypeStruct((S, D), BF),
        in_specs=[hbm_spec] * 6,
        out_specs=hbm_spec,
        scratch_shapes=[
            pltpu.VMEM((S, D), BF),
            pltpu.VMEM((D, 3 * D), BF),
            pltpu.VMEM((D, D), BF),
            pltpu.VMEM((2 * FF, D), BF),
            pltpu.VMEM((FF, D), BF),
            pltpu.VMEM((S, D), BF),
            pltpu.VMEM((S // 2, D), U32),
            pltpu.VMEM((S // 16, D), U32),
            pltpu.VMEM((H, S // 2, 128), U32),
            pltpu.VMEM((H, S // 16, 128), U32),
            pltpu.VMEM((H, 32, S), BF),
            pltpu.VMEM((H, 8, S), F32),
            pltpu.VMEM((D, S), F32),
            pltpu.VMEM((H, 24, S), F32),
            pltpu.VMEM((NKB + NQB, 8, 128), U32),
            pltpu.VMEM((8, 8, 128), F32),
            pltpu.VMEM((CK, TQ), F32),
            pltpu.VMEM((24, TQ), F32),
            pltpu.VMEM((8, TQ), F32),
            pltpu.VMEM((H, 24, S), F32),
            pltpu.VMEM((2, TM3, D), BF),
            pltpu.VMEM((TM3, D), F32),
            pltpu.VMEM((TM3, D), BF),
            pltpu.SemaphoreType.DMA((S // TM1,)),
            pltpu.SemaphoreType.DMA((9,)),
            pltpu.SemaphoreType.DMA((2,)),
        ],
        compiler_params=pltpu.CompilerParams(vmem_limit_bytes=110 * 1024 * 1024),
    )(x2, A_wqkv, A_wo, B_w_gate.T, B_w_up.T, B_w_down)
    return out.reshape(1, S, D)
```

```python
import math
import jax
import jax.numpy as jnp
from jax import lax
import jax.experimental.pallas as pl
import jax.experimental.pallas.tpu as pltpu

S = 2048
D = 640
H = 32
DH = 20
FF = 1728
TQ = 512
CK = 128
NC = S // CK
NU = S // TQ
NL = TQ // 128
TM1 = 512
TM3 = 256
FM = (FF // 128) * 128
FT = FF - FM
EPS = 1e-5
QSCALE = (DH ** -0.5) * math.log2(math.e)

VG = (2, 12)
MG = tuple(g for g in range(15, -1, -1) if g not in VG)
KPERM = MG + VG
RELAX = frozenset((NU - 1, c) for c in range(9, NC))
RORDER = (0, 7, 1, 2, 3, 4, 5, 6)
NKB = NC * len(VG) * DH

BF = jnp.bfloat16
F32 = jnp.float32
U32 = jnp.uint32
NT = (((1,), (1,)), ((), ()))
HI16 = 0xFFFF0000
ONE_BF16_PAIR = 0x3F803F80
L_MAX = 2.0 ** 80
L_MIN = 2.0 ** -60


def _layernorm(x):
    m = jnp.mean(x, axis=-1, keepdims=True)
    xc = x - m
    v = jnp.mean(xc * xc, axis=-1, keepdims=True)
    return xc * lax.rsqrt(v + EPS)


def _layernorm_bf16(x, chunk=64):
    parts = [_layernorm(x[r:r + chunk, :]).astype(BF) for r in range(0, x.shape[0], chunk)]
    return jnp.concatenate(parts, axis=0)


def _row_slice(i, n):
    if isinstance(i, int):
        return pl.ds(i * n, n)
    return pl.ds(pl.multiple_of(i * n, n), n)


def _kb_at(c, j, d):
    n = (c * len(VG) + j) * DH + d
    return (n // NL, slice(None), slice((n % NL) * 128, (n % NL + 1) * 128))


def _qb_at(u, d):
    return NKB // NL + u * DH + d


def _lane_window(arr, start, lane):
    g, rho = start // 128, start % 128
    src = arr[:, g * 128:(g + 1) * 128]
    if rho + 32 > 128 and g + 1 < D // 128:
        src = jnp.where(lane >= 64, src, arr[:, (g + 1) * 128:(g + 2) * 128])
    if rho:
        src = pltpu.roll(src, 128 - rho, 1)
    return src


def _kernel(x_hbm, wqkv_hbm, wo_hbm, wg_hbm, wu_hbm, wd_hbm, out_hbm,
            x_v, wqkv_v, wo_v, wgu_v, wd_v, xn_buf, kperm, kcross, kh, kx, qa, negm, q32, vt,
            vb, fence, ctile, cacc, chk, s_all, otp, out_v, h_buf, hn_buf,
            x_sems, w_sems, out_sems):
    n1 = S // TM1

    def x_copy(i):
        rows = _row_slice(i, TM1)
        return pltpu.make_async_copy(x_hbm.at[rows, :], x_v.at[rows, :], x_sems.at[i])

    srcs = (wqkv_hbm.at[:, pl.ds(0, D)], wqkv_hbm.at[:, pl.ds(D, D)], wqkv_hbm.at[:, pl.ds(2 * D, D)],
            wo_hbm, wd_hbm,
            wg_hbm.at[pl.ds(0, FM), :], wu_hbm.at[pl.ds(0, FM), :],
            wg_hbm.at[pl.ds(FM, FT), :], wu_hbm.at[pl.ds(FM, FT), :])
    dsts = (wqkv_v.at[:, pl.ds(0, D)], wqkv_v.at[:, pl.ds(D, D)], wqkv_v.at[:, pl.ds(2 * D, D)],
            wo_v, wd_v,
            wgu_v.at[pl.ds(0, FM), :], wgu_v.at[pl.ds(FM, FM), :],
            wgu_v.at[pl.ds(2 * FM, FT), :], wgu_v.at[pl.ds(2 * FM + FT, FT), :])
    w_copies = [pltpu.make_async_copy(s_, d_, w_sems.at[i])
                for i, (s_, d_) in enumerate(zip(srcs, dsts))]
    WQ, WK, WV = 0, 1, 2
    x_copy(0).start()
    w_copies[WK].start()
    x_copy(0).wait()
    w_copies[WQ].start()

    def ln_rows(i):
        return _layernorm_bf16(x_v[_row_slice(i, TM1), :].astype(F32))

    def proj_k(i, xn):
        k = jnp.dot(xn, wqkv_v[:, D:2 * D], preferred_element_type=F32)
        grp = lambda c, g: k[c * CK + g * 8:c * CK + g * 8 + 8, :]
        cpb = TM1 // CK
        kp = jnp.concatenate([grp(c, g) for c in range(cpb) for g in KPERM], axis=0).astype(BF)
        kperm[_row_slice(i, TM1 // 2), :] = pltpu.bitcast(kp, U32)
        lo = jnp.concatenate([grp(c, VG[0]) for c in range(cpb)], axis=0).astype(BF).astype(F32)
        hi = jnp.concatenate([grp(c, VG[1]) for c in range(cpb)], axis=0).astype(BF).astype(F32)
        kcross[_row_slice(i, cpb * 8), :] = ((pltpu.bitcast(lo, U32) >> 16)
                                             | (pltpu.bitcast(hi, U32) & jnp.uint32(HI16)))

    xn_buf[...] = ln_rows(0)
    w_copies[WK].wait()
    w_copies[WV].start()
    x_copy(1).start()
    proj_k(0, xn_buf[...])
    w_copies[WQ].wait()
    w_copies[WV].wait()
    for i in range(2, n1):
        x_copy(i).start()

    def gen_kb(h, c):
        kk = kx[h, c * 8:(c + 1) * 8, :]
        for d in range(DH):
            w = jnp.broadcast_to(kk[:, d:d + 1], (8, 128))
            vb[_kb_at(c, 0, d)] = pltpu.bitcast(w << 16, F32)
            vb[_kb_at(c, 1, d)] = pltpu.bitcast(w & jnp.uint32(HI16), F32)

    def gen_qb(h, u, ds=range(DH)):
        for d in ds:
            qq = jnp.broadcast_to(q32[pl.ds(DH * h + d, 1), u * TQ:(u + 1) * TQ], (8, TQ))
            vb[_qb_at(u, d)] = qq
        return qq

    def qv_step(i, carry):
        last = isinstance(i, int)
        if not last:
            x_copy(i + 1).wait()

            @pl.when(i == 1)
            def _():
                for cp in w_copies[3:]:
                    cp.start()

        rows = _row_slice(i, TM1)
        xn = xn_buf[...]
        prow = _row_slice(i, TM1 // 2)
        xrow = _row_slice(i, TM1 // 16)
        kp = kperm[prow, :]
        kc = kcross[xrow, :]
        lane_p = lax.broadcasted_iota(jnp.int32, (TM1 // 2, 128), 1)
        lane_x = lax.broadcasted_iota(jnp.int32, (TM1 // 16, 128), 1)
        for h in range(H):
            w0 = (DH * h // 16) * 16
            rstar = (DH * h - w0 + DH) % 32
            win = _lane_window(kp, w0, lane_p)
            kh[h, prow, :] = jnp.where(lane_p == rstar, jnp.uint32(ONE_BF16_PAIR), win)
            kx[h, xrow, :] = _lane_window(kc, DH * h, lane_x)
        q_t = jnp.dot(xn, wqkv_v[:, 0:D], preferred_element_type=F32).T
        q_t = (q_t * QSCALE).astype(BF).astype(F32)
        q32[:, rows] = q_t
        row32 = lax.broadcasted_iota(jnp.int32, (32, TM1), 0)
        row8 = lax.broadcasted_iota(jnp.int32, (8, TM1), 0)
        for h in range(H):
            w0 = (DH * h // 16) * 16
            off = DH * h - w0
            qw = jnp.where((row32 >= off) & (row32 < off + DH), q_t[w0:w0 + 32, :], 0.0)
            ksub = pltpu.bitcast(kh[h, 0:8, :], BF)[:, 0:32]
            msub = jnp.max(jnp.dot(ksub, qw.astype(BF), preferred_element_type=F32),
                           axis=0, keepdims=True)
            nm = jnp.broadcast_to(-(msub.astype(BF).astype(F32)), (8, TM1))
            rstar = (off + DH) % 32
            t0 = (rstar // 8) * 8
            tiles = [qw[r:r + 8, :] for r in range(0, 32, 8)]
            tiles[t0 // 8] = jnp.where(row8 == rstar - t0, nm, tiles[t0 // 8])
            qa[h, :, rows] = jnp.concatenate(tiles, axis=0).astype(BF)
            negm[h, :, rows] = nm
        if last:
            for u in range(NU):
                gen_qb(0, u)
            for c in range(NC):
                gen_kb(0, c)
        v_t = jnp.dot(xn, wqkv_v[:, 2 * D:3 * D], preferred_element_type=F32).T
        row24 = lax.broadcasted_iota(jnp.int32, (24, TM1), 0)
        for h in range(H):
            v0 = (DH * h // 8) * 8
            ones_row = DH if DH * h == v0 else 0
            vw = v_t[v0:v0 + 24, :].astype(BF).astype(F32)
            vt[h, :, rows] = jnp.where(row24 == ones_row, 1.0, vw)
        if not last:
            xn_next = ln_rows(i + 1)
            proj_k(i + 1, xn_next)
            xn_buf[...] = xn_next
        return carry

    lax.fori_loop(0, n1 - 1, qv_step, 0)
    qv_step(n1 - 1, 0)
    for cp in w_copies[3:]:
        cp.wait()

    def vpu_group(u, c, j, nm):
        acc = nm
        for d in range(DH):
            kb = vb[_kb_at(c, j, d)]
            acc = acc + jnp.concatenate([kb] * NL, axis=1) * vb[_qb_at(u, d)]
        return acc

    def finish_item(hh, cols, acc):
        den = jnp.where(hh % 2 == 0, acc[DH:DH + 1, :], acc[0:1, :])
        otp[hh, :, cols] = acc * (1.0 / den)
        return den

    def pv_step(hh, u, c, tile, acc, never):
        acc = acc + jnp.dot(vt[hh, :, c * CK:(c + 1) * CK], jnp.exp2(tile), preferred_element_type=F32)
        if c == NC - 1:
            den = finish_item(hh, slice(u * TQ, (u + 1) * TQ), acc)
            z = acc * 0.0
            den8 = jnp.broadcast_to(den, (8, TQ))
            chk[0:8, :] = chk[0:8, :] + ((z[0:8] + z[8:16]) + z[16:24])
            chk[8:16, :] = jnp.maximum(chk[8:16, :], den8)
            chk[16:24, :] = jnp.minimum(chk[16:24, :], den8)
            acc = jnp.where(never, acc, 0.0)
        return acc

    def head_step(h, carry):
        hp = (h + H - 1) % H
        hn = (h + 1) % H
        never = h < 0
        acc = cacc[...]
        pend = None
        last_use = {c: max(u for u in range(NU) if (u, c) not in RELAX) for c in range(NC)}
        for u in range(NU):
            cols = slice(u * TQ, (u + 1) * TQ)
            qw = qa[h, :, cols]
            nm = negm[h, :, cols]
            for c in range(NC):
                if (u, c) in RELAX:
                    kk = jnp.concatenate([kh[h, c * 64 + v * 8:c * 64 + v * 8 + 8, :] for v in RORDER], axis=0)
                    s = jnp.dot(pltpu.bitcast(kk, BF)[:, 0:32], qw, preferred_element_type=F32)
                    gord = [KPERM[2 * v + e] for v in RORDER for e in range(2)]
                    g8 = {g: s[i * 8:(i + 1) * 8] for i, g in enumerate(gord)}
                else:
                    km = pltpu.bitcast(kh[h, c * 64:c * 64 + len(MG) * 4, :], BF)[:, 0:32]
                    s = jnp.dot(km, qw, preferred_element_type=F32)
                    g8 = {g: s[i * 8:(i + 1) * 8] for i, g in enumerate(MG)}
                    for j, g in enumerate(VG):
                        nmj = nm
                        dpin = 2 * c + j
                        if u > 0 and dpin < DH:
                            nmj = jnp.where(never, gen_qb(hn, u - 1, [dpin]), nm)
                        g8[g] = vpu_group(u, c, j, nmj)
                        fence[c % 8] = nm[:, 0:128]
                if u == last_use[c]:
                    gen_kb(hn, c)
                if pend is None:
                    acc = pv_step(hp, NU - 1, NC - 1, ctile[...], acc, never)
                else:
                    acc = pv_step(h, pend[0], pend[1], pend[2], acc, never)
                pend = (u, c, jnp.concatenate([g8[g] for g in range(16)], axis=0))
        gen_qb(hn, NU - 1)
        done = [2 * c + j for c in range(NC) for j in range(2) if (NU - 1, c) not in RELAX]
        rest = [d for d in range(DH) if d not in done]
        if rest:
            gen_qb(hn, NU - 2, rest)
        ctile[...] = pend[2]
        cacc[...] = acc
        return carry

    def exact_item(it, carry):
        h = it // NU
        cols = pl.ds(pl.multiple_of((it % NU) * TQ, TQ), TQ)
        rstar = ((4 * h) % 16 + DH) % 32
        row32 = lax.broadcasted_iota(jnp.int32, (32, TQ), 0)
        qw = jnp.where(row32 == rstar, 0.0, qa[h, :, cols].astype(F32)).astype(BF)

        def scores(c, mx):
            kc = pltpu.bitcast(kh[h, pl.ds(pl.multiple_of(c * 64, 64), 64), :], BF)[:, 0:32]
            s = jnp.dot(kc, qw, preferred_element_type=F32)
            g8 = {g: s[i * 8:(i + 1) * 8] for i, g in enumerate(KPERM)}
            s_all[_row_slice(c, CK), :] = jnp.concatenate([g8[g] for g in range(16)], axis=0)
            return jnp.maximum(mx, jnp.max(s, axis=0, keepdims=True))

        m = lax.fori_loop(0, NC, scores, jnp.full((1, TQ), -jnp.inf, F32))

        def weighted(c, acc):
            p = jnp.exp2(s_all[_row_slice(c, CK), :] - m)
            return acc + jnp.dot(vt[h, :, _row_slice(c, CK)], p, preferred_element_type=F32)

        acc = lax.fori_loop(0, NC, weighted, jnp.zeros((24, TQ), F32))
        finish_item(h, cols, acc)
        cacc[...] = acc
        return carry

    def stage_a(i):
        rows = _row_slice(i, TM3)
        sub = lax.broadcasted_iota(jnp.int32, (8, TM3), 0)
        parts = []
        for pr in range(H // 2):
            ev = otp[2 * pr, :, rows]
            od = otp[2 * pr + 1, :, rows]
            parts += [ev[0:16, :], jnp.where(sub < 4, ev[16:24, :], od[0:8, :]), od[8:24, :]]
        o = jnp.concatenate(parts, axis=0).T.astype(BF)
        hres = x_v[rows, :].astype(F32) + jnp.dot(o, wo_v[...], preferred_element_type=F32)
        return hres, _layernorm_bf16(hres)

    def store_a(res):
        h_buf[...] = res[0]
        hn_buf[...] = res[1]

    def attention_pass(attempt, unsafe):
        @pl.when(unsafe > 0.0)
        def _():
            @pl.when(attempt == 0)
            def _():
                lax.fori_loop(0, H, head_step, 0)

            @pl.when(attempt > 0)
            def _():
                lax.fori_loop(0, H * NU, exact_item, 0)
                ctile[...] = jnp.full(ctile.shape, -1e30, F32)

            pv_step(H - 1, NU - 1, NC - 1, ctile[...], cacc[...], attempt < 0)
            store_a(stage_a(0))

        ok = (chk[0:8, :] == 0.0) & (chk[8:16, :] <= L_MAX) & (chk[16:24, :] >= L_MIN)
        return jnp.max(jnp.where(ok, 0.0, 1.0))

    ctile[...] = jnp.zeros(ctile.shape, F32)
    cacc[...] = jnp.ones(cacc.shape, F32)
    chk[0:8, :] = jnp.zeros((8, TQ), F32)
    chk[8:24, :] = jnp.ones((16, TQ), F32)
    lax.fori_loop(0, 2, attention_pass, jnp.float32(1.0))

    n3 = S // TM3

    def out_copy(i, slot):
        return pltpu.make_async_copy(out_v.at[slot], out_hbm.at[_row_slice(i, TM3), :],
                                     out_sems.at[slot])

    def ffn_step(i, carry):
        last = isinstance(i, int)
        slot = i % 2

        if last:
            out_copy(i - 2, slot).wait()
        else:
            @pl.when(i >= 2)
            def _():
                out_copy(i - 2, slot).wait()

        gu = lax.dot_general(hn_buf[...], wgu_v[...], NT, preferred_element_type=F32)
        g = gu[:, 0:FM]
        act = (g * jax.nn.sigmoid(g) * gu[:, FM:2 * FM]).astype(BF)
        gt = gu[:, 2 * FM:2 * FM + FT]
        actt = (gt * jax.nn.sigmoid(gt) * gu[:, 2 * FM + FT:2 * FF]).astype(BF)
        nxt = None if last else stage_a(i + 1)
        y = (h_buf[...] + jnp.dot(act, wd_v[0:FM, :], preferred_element_type=F32)
             + jnp.dot(actt, wd_v[FM:FF, :], preferred_element_type=F32))
        out_v[slot] = y.astype(BF)
        out_copy(i, slot).start()
        if not last:
            store_a(nxt)
        return carry

    lax.fori_loop(0, n3 - 1, ffn_step, 0)
    ffn_step(n3 - 1, 0)
    out_copy(n3 - 2, (n3 - 2) % 2).wait()
    out_copy(n3 - 1, (n3 - 1) % 2).wait()


@jax.jit
def pallas_sequential_preLN__mha_block__swiglu_ffn__prompt_kernel(
    A_x: jax.Array,
    A_wqkv: jax.Array,
    A_wo: jax.Array,
    B_x: jax.Array,
    B_w_gate: jax.Array,
    B_w_up: jax.Array,
    B_w_down: jax.Array,
):
    del B_x
    x2 = A_x.reshape(S, D)
    hbm_spec = pl.BlockSpec(memory_space=pltpu.HBM)
    out = pl.pallas_call(
        _kernel,
        out_shape=jax.ShapeDtypeStruct((S, D), BF),
        in_specs=[hbm_spec] * 6,
        out_specs=hbm_spec,
        scratch_shapes=[
            pltpu.VMEM((S, D), BF),
            pltpu.VMEM((D, 3 * D), BF),
            pltpu.VMEM((D, D), BF),
            pltpu.VMEM((2 * FF, D), BF),
            pltpu.VMEM((FF, D), BF),
            pltpu.VMEM((TM1, D), BF),
            pltpu.VMEM((S // 2, D), U32),
            pltpu.VMEM((S // 16, D), U32),
            pltpu.VMEM((H, S // 2, 128), U32),
            pltpu.VMEM((H, S // 16, 128), U32),
            pltpu.VMEM((H, 32, S), BF),
            pltpu.VMEM((H, 8, S), F32),
            pltpu.VMEM((D, S), F32),
            pltpu.VMEM((H, 24, S), F32),
            pltpu.VMEM((NKB // NL + NU * DH, 8, TQ), F32),
            pltpu.VMEM((8, 8, 128), F32),
            pltpu.VMEM((CK, TQ), F32),
            pltpu.VMEM((24, TQ), F32),
            pltpu.VMEM((24, TQ), F32),
            pltpu.VMEM((S, TQ), F32),
            pltpu.VMEM((H, 24, S), F32),
            pltpu.VMEM((2, TM3, D), BF),
            pltpu.VMEM((TM3, D), F32),
            pltpu.VMEM((TM3, D), BF),
            pltpu.SemaphoreType.DMA((S // TM1,)),
            pltpu.SemaphoreType.DMA((9,)),
            pltpu.SemaphoreType.DMA((2,)),
        ],
        compiler_params=pltpu.CompilerParams(vmem_limit_bytes=110 * 1024 * 1024),
    )(x2, A_wqkv, A_wo, B_w_gate.T, B_w_up.T, B_w_down)
    return out.reshape(1, S, D)
```

```python
import math
import jax
import jax.numpy as jnp
from jax import lax
import jax.experimental.pallas as pl
import jax.experimental.pallas.tpu as pltpu

S = 2048
D = 640
H = 32
DH = 20
FF = 1728
TQ = 512
CK = 128
NC = S // CK
NU = S // TQ
NL = TQ // 128
TM1 = 512
TM3 = 256
FM = (FF // 128) * 128
FT = FF - FM
EPS = 1e-5
QSCALE = (DH ** -0.5) * math.log2(math.e)

VG = (4, 14)
MG = tuple(g for g in range(15, -1, -1) if g not in VG)
KPERM = MG + VG
RELAX = frozenset((NU - 1, c) for c in range(10, 14))
RORDER = (7, 0, 1, 2, 3, 4, 5, 6)
NKB = NC * len(VG) * DH

BF = jnp.bfloat16
F32 = jnp.float32
U32 = jnp.uint32
NT = (((1,), (1,)), ((), ()))
HI16 = 0xFFFF0000
ONE_BF16_PAIR = 0x3F803F80
L_MAX = 2.0 ** 80
L_MIN = 2.0 ** -20


def _layernorm(x):
    m = jnp.mean(x, axis=-1, keepdims=True)
    xc = x - m
    v = jnp.mean(xc * xc, axis=-1, keepdims=True)
    return xc * lax.rsqrt(v + EPS)


def _layernorm_bf16(x, chunk=64):
    parts = [_layernorm(x[r:r + chunk, :]).astype(BF) for r in range(0, x.shape[0], chunk)]
    return jnp.concatenate(parts, axis=0)


def _row_slice(i, n):
    if isinstance(i, int):
        return pl.ds(i * n, n)
    return pl.ds(pl.multiple_of(i * n, n), n)


def _kb_at(c, j, d):
    n = (c * len(VG) + j) * DH + d
    return (n // NL, slice(None), slice((n % NL) * 128, (n % NL + 1) * 128))


def _qb_at(u, d):
    return NKB // NL + u * DH + d


def _lane_window(arr, start, lane):
    g, rho = start // 128, start % 128
    src = arr[:, g * 128:(g + 1) * 128]
    if rho + 32 > 128 and g + 1 < D // 128:
        src = jnp.where(lane >= 64, src, arr[:, (g + 1) * 128:(g + 2) * 128])
    if rho:
        src = pltpu.roll(src, 128 - rho, 1)
    return src


def _kernel(x_hbm, wqkv_hbm, wo_hbm, wg_hbm, wu_hbm, wd_hbm, out_hbm,
            x_v, wqkv_v, wo_v, wgu_v, wd_v, xn_buf, kperm, kcross, kh, kx, qa, negm, q32, vt,
            vb, fence, ctile, cacc, chk, s_all, otp, out_v, h_buf, hn_buf,
            x_sems, w_sems, out_sems):
    n1 = S // TM1

    def x_copy(i):
        rows = _row_slice(i, TM1)
        return pltpu.make_async_copy(x_hbm.at[rows, :], x_v.at[rows, :], x_sems.at[i])

    srcs = (wqkv_hbm.at[:, pl.ds(0, D)], wqkv_hbm.at[:, pl.ds(D, D)], wqkv_hbm.at[:, pl.ds(2 * D, D)],
            wo_hbm, wd_hbm,
            wg_hbm.at[pl.ds(0, FM), :], wu_hbm.at[pl.ds(0, FM), :],
            wg_hbm.at[pl.ds(FM, FT), :], wu_hbm.at[pl.ds(FM, FT), :])
    dsts = (wqkv_v.at[:, pl.ds(0, D)], wqkv_v.at[:, pl.ds(D, D)], wqkv_v.at[:, pl.ds(2 * D, D)],
            wo_v, wd_v,
            wgu_v.at[pl.ds(0, FM), :], wgu_v.at[pl.ds(FM, FM), :],
            wgu_v.at[pl.ds(2 * FM, FT), :], wgu_v.at[pl.ds(2 * FM + FT, FT), :])
    w_copies = [pltpu.make_async_copy(s_, d_, w_sems.at[i])
                for i, (s_, d_) in enumerate(zip(srcs, dsts))]
    WQ, WK, WV = 0, 1, 2
    x_copy(0).start()
    w_copies[WK].start()
    x_copy(0).wait()
    w_copies[WQ].start()

    def ln_rows(i):
        return _layernorm_bf16(x_v[_row_slice(i, TM1), :].astype(F32))

    def proj_k(i, xn):
        k = jnp.dot(xn, wqkv_v[:, D:2 * D], preferred_element_type=F32)
        grp = lambda c, g: k[c * CK + g * 8:c * CK + g * 8 + 8, :]
        cpb = TM1 // CK
        kp = jnp.concatenate([grp(c, g) for c in range(cpb) for g in KPERM], axis=0).astype(BF)
        kperm[_row_slice(i, TM1 // 2), :] = pltpu.bitcast(kp, U32)
        lo = jnp.concatenate([grp(c, VG[0]) for c in range(cpb)], axis=0).astype(BF).astype(F32)
        hi = jnp.concatenate([grp(c, VG[1]) for c in range(cpb)], axis=0).astype(BF).astype(F32)
        kcross[_row_slice(i, cpb * 8), :] = ((pltpu.bitcast(lo, U32) >> 16)
                                             | (pltpu.bitcast(hi, U32) & jnp.uint32(HI16)))

    xn_buf[...] = ln_rows(0)
    w_copies[WK].wait()
    w_copies[WV].start()
    x_copy(1).start()
    proj_k(0, xn_buf[...])
    w_copies[WQ].wait()
    w_copies[WV].wait()
    for i in range(2, n1):
        x_copy(i).start()

    def gen_kb(h):
        kall = kx[h]
        for d in range(DH):
            w = jnp.broadcast_to(kall[:, d:d + 1], (NC * 8, 128))
            lo = pltpu.bitcast(w << 16, F32)
            hi = pltpu.bitcast(w & jnp.uint32(HI16), F32)
            for c in range(NC):
                vb[_kb_at(c, 0, d)] = lo[c * 8:(c + 1) * 8]
                vb[_kb_at(c, 1, d)] = hi[c * 8:(c + 1) * 8]

    def gen_qb(h, u, ds=range(DH)):
        for d in ds:
            qq = jnp.broadcast_to(q32[pl.ds(DH * h + d, 1), u * TQ:(u + 1) * TQ], (8, TQ))
            vb[_qb_at(u, d)] = qq
        return qq

    def qv_step(i, carry):
        last = isinstance(i, int)
        if not last:
            x_copy(i + 1).wait()

            @pl.when(i == 1)
            def _():
                for cp in w_copies[3:]:
                    cp.start()

        rows = _row_slice(i, TM1)
        xn = xn_buf[...]
        prow = _row_slice(i, TM1 // 2)
        xrow = _row_slice(i, TM1 // 16)
        kp = kperm[prow, :]
        kc = kcross[xrow, :]
        lane_p = lax.broadcasted_iota(jnp.int32, (TM1 // 2, 128), 1)
        lane_x = lax.broadcasted_iota(jnp.int32, (TM1 // 16, 128), 1)
        for h in range(H):
            w0 = (DH * h // 16) * 16
            rstar = (DH * h - w0 + DH) % 32
            win = _lane_window(kp, w0, lane_p)
            kh[h, prow, :] = jnp.where(lane_p == rstar, jnp.uint32(ONE_BF16_PAIR), win)
            kx[h, xrow, :] = _lane_window(kc, DH * h, lane_x)
        q_t = jnp.dot(xn, wqkv_v[:, 0:D], preferred_element_type=F32).T
        q_t = (q_t * QSCALE).astype(BF).astype(F32)
        q32[:, rows] = q_t
        row32 = lax.broadcasted_iota(jnp.int32, (32, TM1), 0)
        row8 = lax.broadcasted_iota(jnp.int32, (8, TM1), 0)
        for h in range(H):
            w0 = (DH * h // 16) * 16
            off = DH * h - w0
            qw = jnp.where((row32 >= off) & (row32 < off + DH), q_t[w0:w0 + 32, :], 0.0)
            ksub = pltpu.bitcast(kh[h, 0:8, :], BF)[:, 0:32]
            msub = jnp.max(jnp.dot(ksub, qw.astype(BF), preferred_element_type=F32),
                           axis=0, keepdims=True)
            nm = jnp.broadcast_to(-(msub.astype(BF).astype(F32)), (8, TM1))
            rstar = (off + DH) % 32
            t0 = (rstar // 8) * 8
            tiles = [qw[r:r + 8, :] for r in range(0, 32, 8)]
            tiles[t0 // 8] = jnp.where(row8 == rstar - t0, nm, tiles[t0 // 8])
            qa[h, :, rows] = jnp.concatenate(tiles, axis=0).astype(BF)
            negm[h, :, rows] = nm
        if last:
            for u in range(NU):
                gen_qb(0, u)
            gen_kb(0)
        v_t = jnp.dot(xn, wqkv_v[:, 2 * D:3 * D], preferred_element_type=F32).T
        row24 = lax.broadcasted_iota(jnp.int32, (24, TM1), 0)
        for h in range(H):
            v0 = (DH * h // 8) * 8
            ones_row = DH if DH * h == v0 else 0
            vw = v_t[v0:v0 + 24, :].astype(BF).astype(F32)
            vt[h, :, rows] = jnp.where(row24 == ones_row, 1.0, vw)
        if not last:
            xn_next = ln_rows(i + 1)
            proj_k(i + 1, xn_next)
            xn_buf[...] = xn_next
        return carry

    lax.fori_loop(0, n1 - 1, qv_step, 0)
    qv_step(n1 - 1, 0)
    for cp in w_copies[3:]:
        cp.wait()

    def vpu_group(u, c, j, nm):
        acc = nm
        for d in range(DH):
            kb = vb[_kb_at(c, j, d)]
            acc = acc + jnp.concatenate([kb] * NL, axis=1) * vb[_qb_at(u, d)]
        return acc

    def finish_item(hh, cols, acc):
        den = jnp.where(hh % 2 == 0, acc[DH:DH + 1, :], acc[0:1, :])
        otp[hh, :, cols] = acc * (1.0 / den)
        return den

    def pv_step(hh, u, c, tile, acc, never):
        acc = acc + jnp.dot(vt[hh, :, c * CK:(c + 1) * CK], jnp.exp2(tile), preferred_element_type=F32)
        if c == NC - 1:
            den = finish_item(hh, slice(u * TQ, (u + 1) * TQ), acc)
            z = acc * 0.0
            den8 = jnp.broadcast_to(den, (8, TQ))
            chk[0:8, :] = chk[0:8, :] + ((z[0:8] + z[8:16]) + z[16:24])
            chk[8:16, :] = jnp.maximum(chk[8:16, :], den8)
            chk[16:24, :] = jnp.minimum(chk[16:24, :], den8)
            acc = jnp.where(never, acc, 0.0)
        return acc

    def head_step(h, carry):
        hp = (h + H - 1) % H
        hn = (h + 1) % H
        never = h < 0
        acc = cacc[...]
        pend = None
        for u in range(NU):
            cols = slice(u * TQ, (u + 1) * TQ)
            qw = qa[h, :, cols]
            nm = negm[h, :, cols]
            for c in range(NC):
                if (u, c) in RELAX:
                    kk = jnp.concatenate([kh[h, c * 64 + v * 8:c * 64 + v * 8 + 8, :] for v in RORDER], axis=0)
                    s = jnp.dot(pltpu.bitcast(kk, BF)[:, 0:32], qw, preferred_element_type=F32)
                    gord = [KPERM[2 * v + e] for v in RORDER for e in range(2)]
                    g8 = {g: s[i * 8:(i + 1) * 8] for i, g in enumerate(gord)}
                else:
                    km = pltpu.bitcast(kh[h, c * 64:c * 64 + len(MG) * 4, :], BF)[:, 0:32]
                    s = jnp.dot(km, qw, preferred_element_type=F32)
                    g8 = {g: s[i * 8:(i + 1) * 8] for i, g in enumerate(MG)}
                    for j, g in enumerate(VG):
                        nmj = nm
                        dpin = 2 * c + j
                        if u > 0 and dpin < DH:
                            nmj = jnp.where(never, gen_qb(hn, u - 1, [dpin]), nm)
                        g8[g] = vpu_group(u, c, j, nmj)
                        fence[c % 8] = nm[:, 0:128]
                if (u, c) == (NU - 1, NC - 1):
                    gen_kb(hn)
                if pend is None:
                    acc = pv_step(hp, NU - 1, NC - 1, ctile[...], acc, never)
                else:
                    acc = pv_step(h, pend[0], pend[1], pend[2], acc, never)
                pend = (u, c, jnp.concatenate([g8[g] for g in range(16)], axis=0))
        gen_qb(hn, NU - 1)
        done = [2 * c + j for c in range(NC) for j in range(2) if (NU - 1, c) not in RELAX]
        rest = [d for d in range(DH) if d not in done]
        if rest:
            gen_qb(hn, NU - 2, rest)
        ctile[...] = pend[2]
        cacc[...] = acc
        return carry

    def exact_item(it, carry):
        h = it // NU
        cols = pl.ds(pl.multiple_of((it % NU) * TQ, TQ), TQ)
        rstar = ((4 * h) % 16 + DH) % 32
        row32 = lax.broadcasted_iota(jnp.int32, (32, TQ), 0)
        qw = jnp.where(row32 == rstar, 0.0, qa[h, :, cols].astype(F32)).astype(BF)

        def scores(c, mx):
            kc = pltpu.bitcast(kh[h, pl.ds(pl.multiple_of(c * 64, 64), 64), :], BF)[:, 0:32]
            s = jnp.dot(kc, qw, preferred_element_type=F32)
            g8 = {g: s[i * 8:(i + 1) * 8] for i, g in enumerate(KPERM)}
            s_all[_row_slice(c, CK), :] = jnp.concatenate([g8[g] for g in range(16)], axis=0)
            return jnp.maximum(mx, jnp.max(s, axis=0, keepdims=True))

        m = lax.fori_loop(0, NC, scores, jnp.full((1, TQ), -jnp.inf, F32))

        def weighted(c, acc):
            p = jnp.exp2(s_all[_row_slice(c, CK), :] - m)
            return acc + jnp.dot(vt[h, :, _row_slice(c, CK)], p, preferred_element_type=F32)

        acc = lax.fori_loop(0, NC, weighted, jnp.zeros((24, TQ), F32))
        finish_item(h, cols, acc)
        cacc[...] = acc
        return carry

    def stage_a(i):
        rows = _row_slice(i, TM3)
        sub = lax.broadcasted_iota(jnp.int32, (8, TM3), 0)
        parts = []
        for pr in range(H // 2):
            ev = otp[2 * pr, :, rows]
            od = otp[2 * pr + 1, :, rows]
            parts += [ev[0:16, :], jnp.where(sub < 4, ev[16:24, :], od[0:8, :]), od[8:24, :]]
        o = jnp.concatenate(parts, axis=0).T.astype(BF)
        hres = x_v[rows, :].astype(F32) + jnp.dot(o, wo_v[...], preferred_element_type=F32)
        return hres, _layernorm_bf16(hres)

    def store_a(res):
        h_buf[...] = res[0]
        hn_buf[...] = res[1]

    def attention_pass(attempt, unsafe):
        @pl.when(unsafe > 0.0)
        def _():
            @pl.when(attempt == 0)
            def _():
                lax.fori_loop(0, H, head_step, 0)

            @pl.when(attempt > 0)
            def _():
                lax.fori_loop(0, H * NU, exact_item, 0)
                ctile[...] = jnp.full(ctile.shape, -1e30, F32)

            pv_step(H - 1, NU - 1, NC - 1, ctile[...], cacc[...], attempt < 0)
            store_a(stage_a(0))

        ok = (chk[0:8, :] == 0.0) & (chk[8:16, :] <= L_MAX) & (chk[16:24, :] >= L_MIN)
        return jnp.max(jnp.where(ok, 0.0, 1.0))

    ctile[...] = jnp.zeros(ctile.shape, F32)
    cacc[...] = jnp.ones(cacc.shape, F32)
    chk[0:8, :] = jnp.zeros((8, TQ), F32)
    chk[8:24, :] = jnp.ones((16, TQ), F32)
    lax.fori_loop(0, 2, attention_pass, jnp.float32(1.0))

    n3 = S // TM3

    def out_copy(i, slot):
        return pltpu.make_async_copy(out_v.at[slot], out_hbm.at[_row_slice(i, TM3), :],
                                     out_sems.at[slot])

    def ffn_step(i, carry):
        last = isinstance(i, int)
        slot = i % 2

        if last:
            out_copy(i - 2, slot).wait()
        else:
            @pl.when(i >= 2)
            def _():
                out_copy(i - 2, slot).wait()

        gu = lax.dot_general(hn_buf[...], wgu_v[...], NT, preferred_element_type=F32)
        g = gu[:, 0:FM]
        act = (g * jax.nn.sigmoid(g) * gu[:, FM:2 * FM]).astype(BF)
        gt = gu[:, 2 * FM:2 * FM + FT]
        actt = (gt * jax.nn.sigmoid(gt) * gu[:, 2 * FM + FT:2 * FF]).astype(BF)
        nxt = None if last else stage_a(i + 1)
        y = (h_buf[...] + jnp.dot(act, wd_v[0:FM, :], preferred_element_type=F32)
             + jnp.dot(actt, wd_v[FM:FF, :], preferred_element_type=F32))
        out_v[slot] = y.astype(BF)
        out_copy(i, slot).start()
        if not last:
            store_a(nxt)
        return carry

    lax.fori_loop(0, n3 - 1, ffn_step, 0)
    ffn_step(n3 - 1, 0)
    out_copy(n3 - 2, (n3 - 2) % 2).wait()
    out_copy(n3 - 1, (n3 - 1) % 2).wait()


@jax.jit
def pallas_sequential_preLN__mha_block__swiglu_ffn__prompt_kernel(
    A_x: jax.Array,
    A_wqkv: jax.Array,
    A_wo: jax.Array,
    B_x: jax.Array,
    B_w_gate: jax.Array,
    B_w_up: jax.Array,
    B_w_down: jax.Array,
):
    del B_x
    x2 = A_x.reshape(S, D)
    hbm_spec = pl.BlockSpec(memory_space=pltpu.HBM)
    out = pl.pallas_call(
        _kernel,
        out_shape=jax.ShapeDtypeStruct((S, D), BF),
        in_specs=[hbm_spec] * 6,
        out_specs=hbm_spec,
        scratch_shapes=[
            pltpu.VMEM((S, D), BF),
            pltpu.VMEM((D, 3 * D), BF),
            pltpu.VMEM((D, D), BF),
            pltpu.VMEM((2 * FF, D), BF),
            pltpu.VMEM((FF, D), BF),
            pltpu.VMEM((TM1, D), BF),
            pltpu.VMEM((S // 2, D), U32),
            pltpu.VMEM((S // 16, D), U32),
            pltpu.VMEM((H, S // 2, 128), U32),
            pltpu.VMEM((H, S // 16, 128), U32),
            pltpu.VMEM((H, 32, S), BF),
            pltpu.VMEM((H, 8, S), F32),
            pltpu.VMEM((D, S), F32),
            pltpu.VMEM((H, 24, S), F32),
            pltpu.VMEM((NKB // NL + NU * DH, 8, TQ), F32),
            pltpu.VMEM((8, 8, 128), F32),
            pltpu.VMEM((CK, TQ), F32),
            pltpu.VMEM((24, TQ), F32),
            pltpu.VMEM((24, TQ), F32),
            pltpu.VMEM((S, TQ), F32),
            pltpu.VMEM((H, 24, S), F32),
            pltpu.VMEM((2, TM3, D), BF),
            pltpu.VMEM((TM3, D), F32),
            pltpu.VMEM((TM3, D), BF),
            pltpu.SemaphoreType.DMA((S // TM1,)),
            pltpu.SemaphoreType.DMA((9,)),
            pltpu.SemaphoreType.DMA((2,)),
        ],
        compiler_params=pltpu.CompilerParams(vmem_limit_bytes=110 * 1024 * 1024),
    )(x2, A_wqkv, A_wo, B_w_gate.T, B_w_up.T, B_w_down)
    return out.reshape(1, S, D)
```

```python
import math
import jax
import jax.numpy as jnp
from jax import lax
import jax.experimental.pallas as pl
import jax.experimental.pallas.tpu as pltpu

S = 2048
D = 640
H = 32
DH = 20
FF = 1728
TQ = 512
CK = 128
NC = S // CK
NU = S // TQ
NL = TQ // 128
TM1 = 512
TM3 = 256
FM = (FF // 128) * 128
FT = FF - FM
EPS = 1e-5
QSCALE = (DH ** -0.5) * math.log2(math.e)

VG = (2, 10)
MG = tuple(g for g in range(15, -1, -1) if g not in VG)
KPERM = MG + VG
RELAX = frozenset((NU - 1, c) for c in range(10, 14))
RORDER = (0, 1, 7, 2, 3, 4, 5, 6)
NKB = NC * len(VG) * DH

BF = jnp.bfloat16
F32 = jnp.float32
U32 = jnp.uint32
NT = (((1,), (1,)), ((), ()))
HI16 = 0xFFFF0000
ONE_BF16_PAIR = 0x3F803F80
L_MAX = 2.0 ** 80
L_MIN = 2.0 ** -20


def _layernorm(x):
    m = jnp.mean(x, axis=-1, keepdims=True)
    xc = x - m
    v = jnp.mean(xc * xc, axis=-1, keepdims=True)
    return xc * lax.rsqrt(v + EPS)


def _layernorm_bf16(x, chunk=64):
    parts = [_layernorm(x[r:r + chunk, :]).astype(BF) for r in range(0, x.shape[0], chunk)]
    return jnp.concatenate(parts, axis=0)


def _row_slice(i, n):
    if isinstance(i, int):
        return pl.ds(i * n, n)
    return pl.ds(pl.multiple_of(i * n, n), n)


def _kb_at(c, j, d):
    n = (c * len(VG) + j) * DH + d
    return (n // NL, slice(None), slice((n % NL) * 128, (n % NL + 1) * 128))


def _qb_at(u, d):
    return NKB // NL + u * DH + d


def _lane_window(arr, start, lane):
    g, rho = start // 128, start % 128
    src = arr[:, g * 128:(g + 1) * 128]
    if rho + 32 > 128 and g + 1 < D // 128:
        src = jnp.where(lane >= 64, src, arr[:, (g + 1) * 128:(g + 2) * 128])
    if rho:
        src = pltpu.roll(src, 128 - rho, 1)
    return src


def _kernel(x_hbm, wqkv_hbm, wo_hbm, wg_hbm, wu_hbm, wd_hbm, out_hbm,
            x_v, wqkv_v, wo_v, wgu_v, wd_v, xn_buf, kperm, kcross, kh, kx, qa, negm, q32, vt,
            vb, fence, ctile, cacc, chk, s_all, otp, out_v, h_buf, hn_buf,
            x_sems, w_sems, out_sems):
    n1 = S // TM1

    def x_copy(i):
        rows = _row_slice(i, TM1)
        return pltpu.make_async_copy(x_hbm.at[rows, :], x_v.at[rows, :], x_sems.at[i])

    srcs = (wqkv_hbm.at[:, pl.ds(0, D)], wqkv_hbm.at[:, pl.ds(D, D)], wqkv_hbm.at[:, pl.ds(2 * D, D)],
            wo_hbm, wd_hbm,
            wg_hbm.at[pl.ds(0, FM), :], wu_hbm.at[pl.ds(0, FM), :],
            wg_hbm.at[pl.ds(FM, FT), :], wu_hbm.at[pl.ds(FM, FT), :])
    dsts = (wqkv_v.at[:, pl.ds(0, D)], wqkv_v.at[:, pl.ds(D, D)], wqkv_v.at[:, pl.ds(2 * D, D)],
            wo_v, wd_v,
            wgu_v.at[pl.ds(0, FM), :], wgu_v.at[pl.ds(FM, FM), :],
            wgu_v.at[pl.ds(2 * FM, FT), :], wgu_v.at[pl.ds(2 * FM + FT, FT), :])
    w_copies = [pltpu.make_async_copy(s_, d_, w_sems.at[i])
                for i, (s_, d_) in enumerate(zip(srcs, dsts))]
    WQ, WK, WV = 0, 1, 2
    x_copy(0).start()
    w_copies[WK].start()
    x_copy(0).wait()
    w_copies[WQ].start()

    def ln_rows(i):
        return _layernorm_bf16(x_v[_row_slice(i, TM1), :].astype(F32))

    def proj_k(i, xn):
        k = jnp.dot(xn, wqkv_v[:, D:2 * D], preferred_element_type=F32)
        grp = lambda c, g: k[c * CK + g * 8:c * CK + g * 8 + 8, :]
        cpb = TM1 // CK
        kp = jnp.concatenate([grp(c, g) for c in range(cpb) for g in KPERM], axis=0).astype(BF)
        kperm[_row_slice(i, TM1 // 2), :] = pltpu.bitcast(kp, U32)
        lo = jnp.concatenate([grp(c, VG[0]) for c in range(cpb)], axis=0).astype(BF).astype(F32)
        hi = jnp.concatenate([grp(c, VG[1]) for c in range(cpb)], axis=0).astype(BF).astype(F32)
        kcross[_row_slice(i, cpb * 8), :] = ((pltpu.bitcast(lo, U32) >> 16)
                                             | (pltpu.bitcast(hi, U32) & jnp.uint32(HI16)))

    xn_buf[...] = ln_rows(0)
    w_copies[WK].wait()
    w_copies[WV].start()
    x_copy(1).start()
    proj_k(0, xn_buf[...])
    w_copies[WQ].wait()
    w_copies[WV].wait()
    for i in range(2, n1):
        x_copy(i).start()

    def gen_kb(h):
        kall = kx[h]
        for d in range(DH):
            w = jnp.broadcast_to(kall[:, d:d + 1], (NC * 8, 128))
            lo = pltpu.bitcast(w << 16, F32)
            hi = pltpu.bitcast(w & jnp.uint32(HI16), F32)
            for c in range(NC):
                vb[_kb_at(c, 0, d)] = lo[c * 8:(c + 1) * 8]
                vb[_kb_at(c, 1, d)] = hi[c * 8:(c + 1) * 8]

    def gen_qb(h, u, ds=range(DH)):
        for d in ds:
            qq = jnp.broadcast_to(q32[pl.ds(DH * h + d, 1), u * TQ:(u + 1) * TQ], (8, TQ))
            vb[_qb_at(u, d)] = qq
        return qq

    def qv_step(i, carry):
        last = isinstance(i, int)
        if not last:
            x_copy(i + 1).wait()

            @pl.when(i == 1)
            def _():
                for cp in w_copies[3:]:
                    cp.start()

        rows = _row_slice(i, TM1)
        xn = xn_buf[...]
        prow = _row_slice(i, TM1 // 2)
        xrow = _row_slice(i, TM1 // 16)
        kp = kperm[prow, :]
        kc = kcross[xrow, :]
        lane_p = lax.broadcasted_iota(jnp.int32, (TM1 // 2, 128), 1)
        lane_x = lax.broadcasted_iota(jnp.int32, (TM1 // 16, 128), 1)
        for h in range(H):
            w0 = (DH * h // 16) * 16
            rstar = (DH * h - w0 + DH) % 32
            win = _lane_window(kp, w0, lane_p)
            kh[h, prow, :] = jnp.where(lane_p == rstar, jnp.uint32(ONE_BF16_PAIR), win)
            kx[h, xrow, :] = _lane_window(kc, DH * h, lane_x)
        q_t = jnp.dot(xn, wqkv_v[:, 0:D], preferred_element_type=F32).T
        q_t = (q_t * QSCALE).astype(BF).astype(F32)
        q32[:, rows] = q_t
        row32 = lax.broadcasted_iota(jnp.int32, (32, TM1), 0)
        row8 = lax.broadcasted_iota(jnp.int32, (8, TM1), 0)
        for h in range(H):
            w0 = (DH * h // 16) * 16
            off = DH * h - w0
            qw = jnp.where((row32 >= off) & (row32 < off + DH), q_t[w0:w0 + 32, :], 0.0)
            ksub = pltpu.bitcast(kh[h, 0:8, :], BF)[:, 0:32]
            msub = jnp.max(jnp.dot(ksub, qw.astype(BF), preferred_element_type=F32),
                           axis=0, keepdims=True)
            nm = jnp.broadcast_to(-(msub.astype(BF).astype(F32)), (8, TM1))
            rstar = (off + DH) % 32
            t0 = (rstar // 8) * 8
            tiles = [qw[r:r + 8, :] for r in range(0, 32, 8)]
            tiles[t0 // 8] = jnp.where(row8 == rstar - t0, nm, tiles[t0 // 8])
            qa[h, :, rows] = jnp.concatenate(tiles, axis=0).astype(BF)
            negm[h, :, rows] = nm
        if last:
            for u in range(NU):
                gen_qb(0, u)
            gen_kb(0)
        v_t = jnp.dot(xn, wqkv_v[:, 2 * D:3 * D], preferred_element_type=F32).T
        row24 = lax.broadcasted_iota(jnp.int32, (24, TM1), 0)
        for h in range(H):
            v0 = (DH * h // 8) * 8
            ones_row = DH if DH * h == v0 else 0
            vw = v_t[v0:v0 + 24, :].astype(BF).astype(F32)
            vt[h, :, rows] = jnp.where(row24 == ones_row, 1.0, vw)
        if not last:
            xn_next = ln_rows(i + 1)
            proj_k(i + 1, xn_next)
            xn_buf[...] = xn_next
        return carry

    lax.fori_loop(0, n1 - 1, qv_step, 0)
    qv_step(n1 - 1, 0)
    for cp in w_copies[3:]:
        cp.wait()

    def vpu_group(u, c, j, nm):
        acc = nm
        for d in range(DH):
            kb = vb[_kb_at(c, j, d)]
            acc = acc + jnp.concatenate([kb] * NL, axis=1) * vb[_qb_at(u, d)]
        return acc

    def pv_step(hh, u, c, tile, acc, never):
        acc = acc + jnp.dot(vt[hh, :, c * CK:(c + 1) * CK], jnp.exp2(tile), preferred_element_type=F32)
        if c == NC - 1:
            otp[hh, :, u * TQ:(u + 1) * TQ] = acc
            acc = jnp.where(never, acc, 0.0)
        return acc

    def head_step(h, carry):
        hp = (h + H - 1) % H
        hn = (h + 1) % H
        never = h < 0
        acc = cacc[...]
        pend = None
        for u in range(NU):
            cols = slice(u * TQ, (u + 1) * TQ)
            qw = qa[h, :, cols]
            nm = negm[h, :, cols]
            for c in range(NC):
                if (u, c) in RELAX:
                    kk = jnp.concatenate([kh[h, c * 64 + v * 8:c * 64 + v * 8 + 8, :] for v in RORDER], axis=0)
                    s = jnp.dot(pltpu.bitcast(kk, BF)[:, 0:32], qw, preferred_element_type=F32)
                    gord = [KPERM[2 * v + e] for v in RORDER for e in range(2)]
                    g8 = {g: s[i * 8:(i + 1) * 8] for i, g in enumerate(gord)}
                else:
                    km = pltpu.bitcast(kh[h, c * 64:c * 64 + len(MG) * 4, :], BF)[:, 0:32]
                    s = jnp.dot(km, qw, preferred_element_type=F32)
                    g8 = {g: s[i * 8:(i + 1) * 8] for i, g in enumerate(MG)}
                    for j, g in enumerate(VG):
                        nmj = nm
                        dpin = 2 * c + j
                        if u > 0 and dpin < DH:
                            nmj = jnp.where(never, gen_qb(hn, u - 1, [dpin]), nm)
                        g8[g] = vpu_group(u, c, j, nmj)
                        fence[c % 8] = nm[:, 0:128]
                if (u, c) == (NU - 1, NC - 1):
                    gen_kb(hn)
                if pend is None:
                    acc = pv_step(hp, NU - 1, NC - 1, ctile[...], acc, never)
                else:
                    acc = pv_step(h, pend[0], pend[1], pend[2], acc, never)
                pend = (u, c, jnp.concatenate([g8[g] for g in range(16)], axis=0))
        gen_qb(hn, NU - 1)
        done = [2 * c + j for c in range(NC) for j in range(2) if (NU - 1, c) not in RELAX]
        rest = [d for d in range(DH) if d not in done]
        if rest:
            gen_qb(hn, NU - 2, rest)
        ctile[...] = pend[2]
        cacc[...] = acc
        return carry

    def exact_item(it, carry):
        h = it // NU
        cols = pl.ds(pl.multiple_of((it % NU) * TQ, TQ), TQ)
        rstar = ((4 * h) % 16 + DH) % 32
        row32 = lax.broadcasted_iota(jnp.int32, (32, TQ), 0)
        qw = jnp.where(row32 == rstar, 0.0, qa[h, :, cols].astype(F32)).astype(BF)

        def scores(c, mx):
            kc = pltpu.bitcast(kh[h, pl.ds(pl.multiple_of(c * 64, 64), 64), :], BF)[:, 0:32]
            s = jnp.dot(kc, qw, preferred_element_type=F32)
            g8 = {g: s[i * 8:(i + 1) * 8] for i, g in enumerate(KPERM)}
            s_all[_row_slice(c, CK), :] = jnp.concatenate([g8[g] for g in range(16)], axis=0)
            return jnp.maximum(mx, jnp.max(s, axis=0, keepdims=True))

        m = lax.fori_loop(0, NC, scores, jnp.full((1, TQ), -jnp.inf, F32))

        def weighted(c, acc):
            p = jnp.exp2(s_all[_row_slice(c, CK), :] - m)
            return acc + jnp.dot(vt[h, :, _row_slice(c, CK)], p, preferred_element_type=F32)

        acc = lax.fori_loop(0, NC, weighted, jnp.zeros((24, TQ), F32))
        otp[h, :, cols] = acc
        cacc[...] = acc
        return carry

    def stage_a(i):
        rows = _row_slice(i, TM3)
        sub = lax.broadcasted_iota(jnp.int32, (8, TM3), 0)
        parts = []
        z, hi, lo = chk[0], chk[1], chk[2]
        for pr in range(H // 2):
            ev = otp[2 * pr, :, rows]
            od = otp[2 * pr + 1, :, rows]
            z = z + (((ev[0:8] + ev[8:16]) + (ev[16:24] + od[0:8])) + (od[8:16] + od[16:24]))
            dens = jnp.where(sub < 4, od[0:8], ev[16:24])
            hi = jnp.maximum(hi, dens)
            lo = jnp.minimum(lo, dens)
            rec = 1.0 / dens
            ev = ev * rec[4:5, :]
            od = od * rec[0:1, :]
            parts += [ev[0:16, :], jnp.where(sub < 4, ev[16:24, :], od[0:8, :]), od[8:24, :]]
        chk[0] = z
        chk[1] = hi
        chk[2] = lo
        o = jnp.concatenate(parts, axis=0).T.astype(BF)
        hres = x_v[rows, :].astype(F32) + jnp.dot(o, wo_v[...], preferred_element_type=F32)
        return hres, _layernorm_bf16(hres)

    def store_a(res):
        h_buf[...] = res[0]
        hn_buf[...] = res[1]

    n3 = S // TM3

    def out_copy(i, slot):
        return pltpu.make_async_copy(out_v.at[slot], out_hbm.at[_row_slice(i, TM3), :],
                                     out_sems.at[slot])

    def ffn_step(i, carry):
        last = isinstance(i, int)
        slot = i % 2

        if last:
            out_copy(i - 2, slot).wait()
        else:
            @pl.when(i >= 2)
            def _():
                out_copy(i - 2, slot).wait()

        gu = lax.dot_general(hn_buf[...], wgu_v[...], NT, preferred_element_type=F32)
        g = gu[:, 0:FM]
        act = (g * jax.nn.sigmoid(g) * gu[:, FM:2 * FM]).astype(BF)
        gt = gu[:, 2 * FM:2 * FM + FT]
        actt = (gt * jax.nn.sigmoid(gt) * gu[:, 2 * FM + FT:2 * FF]).astype(BF)
        nxt = None if last else stage_a(i + 1)
        y = (h_buf[...] + jnp.dot(act, wd_v[0:FM, :], preferred_element_type=F32)
             + jnp.dot(actt, wd_v[FM:FF, :], preferred_element_type=F32))
        out_v[slot] = y.astype(BF)
        out_copy(i, slot).start()
        if not last:
            store_a(nxt)
        return carry

    def full_pass(attempt, unsafe):
        @pl.when(unsafe > 0.0)
        def _():
            @pl.when(attempt == 0)
            def _():
                lax.fori_loop(0, H, head_step, 0)

            @pl.when(attempt > 0)
            def _():
                lax.fori_loop(0, H * NU, exact_item, 0)
                ctile[...] = jnp.full(ctile.shape, -1e30, F32)

            pv_step(H - 1, NU - 1, NC - 1, ctile[...], cacc[...], attempt < 0)
            store_a(stage_a(0))
            lax.fori_loop(0, n3 - 1, ffn_step, 0)
            ffn_step(n3 - 1, 0)

        def check():
            sub = lax.broadcasted_iota(jnp.int32, (8, TM3), 0)
            in_range = (chk[1] <= L_MAX) & (chk[2] >= L_MIN)
            ok = (chk[0] * 0.0 == 0.0) & (in_range | (sub % 4 != 0))
            return jnp.max(jnp.where(ok, 0.0, 1.0))

        flag = lax.cond(attempt == 0, check, lambda: jnp.float32(0.0))

        @pl.when(unsafe > 0.0)
        def _():
            out_copy(n3 - 2, (n3 - 2) % 2).wait()
            out_copy(n3 - 1, (n3 - 1) % 2).wait()

        return flag

    ctile[...] = jnp.zeros(ctile.shape, F32)
    cacc[...] = jnp.ones(cacc.shape, F32)
    chk[...] = jnp.ones(chk.shape, F32)
    lax.fori_loop(0, 2, full_pass, jnp.float32(1.0))


@jax.jit
def pallas_sequential_preLN__mha_block__swiglu_ffn__prompt_kernel(
    A_x: jax.Array,
    A_wqkv: jax.Array,
    A_wo: jax.Array,
    B_x: jax.Array,
    B_w_gate: jax.Array,
    B_w_up: jax.Array,
    B_w_down: jax.Array,
):
    del B_x
    x2 = A_x.reshape(S, D)
    hbm_spec = pl.BlockSpec(memory_space=pltpu.HBM)
    out = pl.pallas_call(
        _kernel,
        out_shape=jax.ShapeDtypeStruct((S, D), BF),
        in_specs=[hbm_spec] * 6,
        out_specs=hbm_spec,
        scratch_shapes=[
            pltpu.VMEM((S, D), BF),
            pltpu.VMEM((D, 3 * D), BF),
            pltpu.VMEM((D, D), BF),
            pltpu.VMEM((2 * FF, D), BF),
            pltpu.VMEM((FF, D), BF),
            pltpu.VMEM((TM1, D), BF),
            pltpu.VMEM((S // 2, D), U32),
            pltpu.VMEM((S // 16, D), U32),
            pltpu.VMEM((H, S // 2, 128), U32),
            pltpu.VMEM((H, S // 16, 128), U32),
            pltpu.VMEM((H, 32, S), BF),
            pltpu.VMEM((H, 8, S), F32),
            pltpu.VMEM((D, S), F32),
            pltpu.VMEM((H, 24, S), F32),
            pltpu.VMEM((NKB // NL + NU * DH, 8, TQ), F32),
            pltpu.VMEM((8, 8, 128), F32),
            pltpu.VMEM((CK, TQ), F32),
            pltpu.VMEM((24, TQ), F32),
            pltpu.VMEM((3, 8, TM3), F32),
            pltpu.VMEM((S, TQ), F32),
            pltpu.VMEM((H, 24, S), F32),
            pltpu.VMEM((2, TM3, D), BF),
            pltpu.VMEM((TM3, D), F32),
            pltpu.VMEM((TM3, D), BF),
            pltpu.SemaphoreType.DMA((S // TM1,)),
            pltpu.SemaphoreType.DMA((9,)),
            pltpu.SemaphoreType.DMA((2,)),
        ],
        compiler_params=pltpu.CompilerParams(vmem_limit_bytes=110 * 1024 * 1024),
    )(x2, A_wqkv, A_wo, B_w_gate.T, B_w_up.T, B_w_down)
    return out.reshape(1, S, D)
```
